```python
import os as _os
_os.environ.setdefault("JAX_PLATFORMS", "cpu")
import jax
import jax.numpy as jnp

def _softmax(x, axis=-1):
    return jax.nn.softmax(x, axis=axis)
def _gelu(x):
    return jax.nn.gelu(x, approximate=True)
def _silu(x):
    return jax.nn.silu(x)
def _sigmoid(x):
    return jax.nn.sigmoid(x)
def _layernorm(x, axis=-1, eps=1e-5):
    m = jnp.mean(x, axis=axis, keepdims=True)
    v = jnp.var(x, axis=axis, keepdims=True)
    return (x - m) / jnp.sqrt(v + eps)
def _scatter_add(tgt, idx, src, axis=0):
    return tgt.at[idx].add(src)
def _segment_sum(src, seg, n):
    return jax.ops.segment_sum(src, seg, n)
class _Rng:
    def __init__(self, key):
        self._k = key
    def _next(self):
        self._k, sub = jax.random.split(self._k)
        return sub
    def normal(self, shape):
        return jax.random.normal(self._next(), shape, dtype=jnp.bfloat16)
    def randint(self, lo, hi, shape):
        return jax.random.randint(self._next(), shape, lo, hi, dtype=jnp.int32)
    def uniform(self, shape, lo=0.0, hi=1.0):
        return jax.random.uniform(self._next(), shape, jnp.bfloat16, lo, hi)
    def permutation(self, n):
        return jax.random.permutation(self._next(), n)


kernel_name = 'gated_mix__sliding_block_cached__swiglu_ffn__decode'

def setup_inputs():
    _rng = _Rng(jax.random.key(int.from_bytes(__import__("os").urandom(4), "little")))
    _w = (lambda a: (lambda t: t.astype(jnp.bfloat16) if jnp.issubdtype(t.dtype, jnp.floating) else t)(jnp.asarray(a)))
    def _A_setup():
        B, Sq, D = 1, 1, 512
        Hq, Hkv, Sk, Dh = 32, 32, 32768, 128
        assert Hq % Hkv == 0, (Hq, Hkv)
        return {
            "x": _w((lambda *s: _rng.normal(s) * 0.05)(B, Sq, D)),
            "k_cache": _w((lambda *s: _rng.normal(s) * 3.2)(B, Hkv, Sk, Dh)),
            "v_cache": _w((lambda *s: _rng.normal(s) * 1.6)(B, Hkv, Sk, Dh)),
            "wq": _w((lambda *s: _rng.normal(s) * 3.2)(D, Hq * Dh) * (D ** -0.5)),
            "wo": _w((lambda *s: _rng.normal(s) * 1.6)(Hq * Dh, D) * ((Hq * Dh) ** -0.5)),
        }
    _A_in = _A_setup()

    def _B_setup():
        B, S, D, F = 1, 1, 512, 1376
        return {
            "x": _w((lambda *s: _rng.normal(s) * 0.05)(B, S, D)),
            "w_gate": _w((lambda *s: _rng.normal(s) * 0.1)(D, F)),
            "w_up": _w((lambda *s: _rng.normal(s) * 0.1)(D, F)),
            "w_down": _w((lambda *s: _rng.normal(s) * 0.1)(F, D)),
        }
    _B_in = _B_setup()

    return {
        "A_x": _A_in["x"],
        "A_k_cache": _A_in["k_cache"],
        "A_v_cache": _A_in["v_cache"],
        "A_wq": _A_in["wq"],
        "A_wo": _A_in["wo"],
        "B_x": _B_in["x"],
        "B_w_gate": _B_in["w_gate"],
        "B_w_up": _B_in["w_up"],
        "B_w_down": _B_in["w_down"],
        "gate_w": _w((lambda *s: _rng.normal(s) * 0.05)(512) * 16.0),
    }

def reference(A_x, A_k_cache, A_v_cache, A_wq, A_wo, B_x, B_w_gate, B_w_up, B_w_down, gate_w):
    def _A_ref(x, k_cache, v_cache, wq, wo):
        B, Sq, D = x.shape
        Hq, Dh = 32, 128
        Hkv, Sk = k_cache.shape[1], k_cache.shape[2]
        W = min(4096, max(256, Sk // 4))
        rep = Hq // Hkv
        q = (lambda x, *d: x.transpose(*d))((x @ wq).reshape(B, Sq, Hq, Dh), 0, 2, 1, 3)
        k = jnp.repeat(k_cache[:, :, Sk - W:, :], rep, axis=1)
        v = jnp.repeat(v_cache[:, :, Sk - W:, :], rep, axis=1)
        scores = jnp.einsum("bhqd,bhkd->bhqk", q, k) * (Dh ** -0.5)
        p = _softmax(scores, axis=-1)
        o = jnp.einsum("bhqk,bhkd->bhqd", p, v)
        return (lambda x, *d: x.transpose(*d))(o, 0, 2, 1, 3).reshape(B, Sq, Hq * Dh) @ wo

    def _B_ref(x, w_gate, w_up, w_down):
        g = _silu(x @ w_gate)
        u = x @ w_up
        return (g * u) @ w_down

    x = A_x
    g = _sigmoid((x * gate_w).sum(-1, keepdims=True))
    a = _A_ref(x, A_k_cache, A_v_cache, A_wq, A_wo)
    b = _B_ref(x, B_w_gate, B_w_up, B_w_down)
    return g * a + (1 - g) * b
```

```python
import functools
import jax
import jax.numpy as jnp
from jax import lax
import jax.experimental.pallas as pl
import jax.experimental.pallas.tpu as pltpu

CFG = dict(BLK=1024, TR=192, NB=6, NTR=4, PT=0, PB=1, NOBC=True, WDT=256)

NT = (((1,), (1,)), ((), ()))


def build(cfg):
    BLK = cfg["BLK"]; TR = cfg["TR"]; NB = cfg["NB"]; NTR = cfg["NTR"]; PT = cfg["PT"]; PB = cfg["PB"]
    WDT = cfg["WDT"]

    def fn(A_x, A_k_cache, A_v_cache, A_wq, A_wo, B_x, B_w_gate, B_w_up, B_w_down, gate_w):
        B, Sq, D = A_x.shape
        _, H, Sk, Dh = A_k_cache.shape
        W = min(4096, max(256, Sk // 4))
        F = B_w_gate.shape[1]
        scale = Dh ** -0.5
        S0 = Sk - W
        NK = W // BLK
        T = 2 * NK
        BR = BLK - TR
        assert NB < T and NTR < T
        QP = D // NK
        OP = Dh // NK
        F2 = F - WDT
        DP = OP
        F1 = F2 - T * DP
        f32 = jnp.float32
        bf16 = jnp.bfloat16

        def kernel(x_hbm, k_hbm, v_hbm, wq_hbm, wo_hbm, wg_hbm, wu_hbm, wd_hbm, gw_hbm, o_hbm,
                   x_v, gw_v, kvbuf, wqbuf, wobuf, wgbuf, wubuf, wdbuf, o_v,
                   sem_misc, sem_b, sem_t, sem_w):
            def kv_src(t):
                return (k_hbm, t) if t < NK else (v_hbm, t - NK)

            def bulk(h, t):
                src, j = kv_src(t)
                return pltpu.make_async_copy(
                    src.at[0, h, pl.ds(S0 + j * BLK, BR), :], kvbuf.at[t, pl.ds(0, BR), :], sem_b.at[t])

            def trk(h, t):
                src, j = kv_src(t)
                return pltpu.make_async_copy(
                    src.at[0, h, pl.ds(S0 + j * BLK + BR, TR), :], kvbuf.at[t, pl.ds(BR, TR), :], sem_t.at[t])

            def aligned(i, n):
                return i if isinstance(i, int) else pl.multiple_of(i, n)

            def wq_piece(hh, j):
                return pltpu.make_async_copy(
                    wq_hbm.at[pl.ds(j * QP, QP), pl.ds(aligned(hh * Dh, Dh), Dh)],
                    wqbuf.at[pl.ds(j * QP, QP), :], sem_w.at[0])

            def wq_wait():
                pltpu.make_async_copy(wqbuf, wqbuf, sem_w.at[0]).wait()

            def wo_piece(hh, slot, j):
                return pltpu.make_async_copy(
                    wo_hbm.at[pl.ds(aligned(hh * Dh + j * OP, OP), OP), :],
                    wobuf.at[slot, pl.ds(j * OP, OP), :], sem_w.at[1 + slot])

            def wo_wait(slot):
                pltpu.make_async_copy(wobuf.at[slot], wobuf.at[slot], sem_w.at[1 + slot]).wait()

            def wd_copy(r0, n, sem):
                return pltpu.make_async_copy(wd_hbm.at[pl.ds(r0, n), :], wdbuf.at[pl.ds(r0, n), :], sem)

            cp_x = pltpu.make_async_copy(x_hbm, x_v, sem_misc.at[0])
            cp_gw = pltpu.make_async_copy(gw_hbm, gw_v, sem_misc.at[1])
            cp_wg = pltpu.make_async_copy(wg_hbm, wgbuf, sem_misc.at[2])
            cp_wu = pltpu.make_async_copy(wu_hbm, wubuf, sem_misc.at[3])
            cp_wd1 = wd_copy(0, F1, sem_misc.at[4])
            cp_wd3 = wd_copy(F2, F - F2, sem_misc.at[5])

            cp_wg.start(priority=PB)
            cp_x.start(priority=PT)
            cp_gw.start(priority=PT)
            for j in range(NK):
                wq_piece(0, j).start(priority=PT)
            cp_wu.start(priority=PB)
            cp_x.wait()
            cp_wd1.start(priority=PB)
            for j in range(NK):
                wo_piece(0, 0, j).start(priority=PT)
            x = x_v[0]
            x8 = jnp.broadcast_to(x, (8, D))
            cp_gw.wait()
            for t in range(NB):
                bulk(0, t).start(priority=PB)
            gw = gw_v[...].reshape(1, D).astype(f32)
            gate = jax.nn.sigmoid(jnp.sum(x.astype(f32) * gw, axis=-1, keepdims=True))
            wq_wait()
            q0 = jnp.dot(x8, wqbuf[...], preferred_element_type=f32).astype(bf16)
            cp_wg.wait()
            if TR:
                for t in range(NTR):
                    trk(0, t).start(priority=PT)
            gt = lax.dot_general(x8, wgbuf[...], NT, preferred_element_type=f32)
            cp_wu.wait()
            u = lax.dot_general(x8, wubuf[...], NT, preferred_element_type=f32)
            hid = (gt * jax.nn.sigmoid(gt) * u).astype(bf16)
            cp_wd1.wait()
            b1 = jnp.dot(hid[:, :F1], wdbuf[pl.ds(0, F1), :], preferred_element_type=f32)
            if TR:
                trk(0, 0).wait()

            def head(h, slot, q, out_acc, last):
                def tick_start(t):
                    bulk(h, t).wait()
                    if TR:
                        tn = t + NTR
                        if tn < T:
                            trk(h, tn).start(priority=PT)
                        elif not last:
                            trk(h + 1, tn - T).start(priority=PT)
                    tn = t + NB
                    if tn < T:
                        bulk(h, tn).start(priority=PB)
                    elif not last:
                        bulk(h + 1, tn - T).start(priority=PB)
                    elif tn == T:
                        cp_wd3.start(priority=PB)

                def tick_mid(t):
                    if TR:
                        if t + 1 < T:
                            trk(h, t + 1).wait()
                        elif not last:
                            trk(h + 1, 0).wait()
                    if last:
                        wd_copy(F1 + t * DP, DP, sem_misc.at[6]).start(priority=PT)
                    elif t < NK:
                        wq_piece(h + 1, t).start(priority=PT)
                    else:
                        wo_piece(h + 1, 1 - slot, t - NK).start(priority=PT)

                ss = []
                for t in range(NK):
                    tick_start(t)
                    ss.append(lax.dot_general(q, kvbuf[t], NT, preferred_element_type=f32))
                    tick_mid(t)
                s = jnp.concatenate(ss, axis=1) * scale
                m = jnp.max(s, axis=-1, keepdims=True)
                p = jnp.exp(s - m)
                l = jnp.sum(p, axis=-1, keepdims=True)
                pb = p.astype(bf16)
                acc = jnp.zeros((8, Dh), f32)
                qn = q
                for j in range(NK):
                    t = NK + j
                    tick_start(t)
                    if j == min(1, NK - 1) and not last:
                        wq_wait()
                        qn = jnp.dot(x8, wqbuf[...], preferred_element_type=f32).astype(bf16)
                    if j == NK - 1:
                        wo_wait(slot)
                    acc = acc + jnp.dot(pb[:, j * BLK:(j + 1) * BLK], kvbuf[t], preferred_element_type=f32)
                    tick_mid(t)
                o = (acc / l).astype(bf16)
                out_acc = out_acc + jnp.dot(o, wobuf[slot], preferred_element_type=f32)
                return qn, out_acc

            def body(h, carry):
                q, out_acc = carry
                return head(h, h % 2, q, out_acc, False)

            q, out_acc = lax.fori_loop(0, H - 1, body, (q0, jnp.zeros((8, D), f32)))
            _, out_acc = head(H - 1, (H - 1) % 2, q, out_acc, True)

            wd_copy(F1, F2 - F1, sem_misc.at[6]).wait()
            cp_wd3.wait()
            b = b1 + jnp.dot(hid[:, F1:], wdbuf[pl.ds(F1, F - F1), :], preferred_element_type=f32)
            res = gate * out_acc + (1.0 - gate) * b
            o_v[0] = res[0:1].astype(o_v.dtype)
            cp_o = pltpu.make_async_copy(o_v, o_hbm, sem_misc.at[7])
            cp_o.start()
            cp_o.wait()

        any_spec = pl.BlockSpec(memory_space=pl.ANY)
        return pl.pallas_call(
            kernel,
            in_specs=[any_spec] * 9,
            out_specs=any_spec,
            out_shape=jax.ShapeDtypeStruct((B, Sq, D), A_x.dtype),
            scratch_shapes=[
                pltpu.VMEM((1, 1, D), bf16), pltpu.VMEM((D,), bf16),
                pltpu.VMEM((T, BLK, Dh), bf16),
                pltpu.VMEM((D, Dh), bf16), pltpu.VMEM((2, Dh, D), bf16),
                pltpu.VMEM((F, D), bf16), pltpu.VMEM((F, D), bf16), pltpu.VMEM((F, D), bf16),
                pltpu.VMEM((1, 1, D), bf16),
                pltpu.SemaphoreType.DMA((8,)), pltpu.SemaphoreType.DMA((T,)),
                pltpu.SemaphoreType.DMA((T,)), pltpu.SemaphoreType.DMA((3,)),
            ],
            compiler_params=pltpu.CompilerParams(vmem_limit_bytes=64 * 1024 * 1024,
                                                 disable_bounds_checks=cfg["NOBC"]),
        )(A_x, A_k_cache, A_v_cache, A_wq, A_wo, B_w_gate.T, B_w_up.T, B_w_down, gate_w)

    return jax.jit(fn)


pallas_gated_mix__sliding_block_cached__swiglu_ffn__decode_kernel = build(CFG)
```

```python
import functools
import jax
import jax.numpy as jnp
from jax import lax
import jax.experimental.pallas as pl
import jax.experimental.pallas.tpu as pltpu

CFG = dict(R=8, NB=6, NOBC=True, NOSC=True, STAG=False)

NT = (((1,), (1,)), ((), ()))
PT, PB = 0, 1


def build(cfg):
    R = cfg["R"]; NB = cfg["NB"]; STAG = cfg["STAG"]

    def fn(A_x, A_k_cache, A_v_cache, A_wq, A_wo, B_x, B_w_gate, B_w_up, B_w_down, gate_w):
        B, Sq, D = A_x.shape
        _, H, Sk, Dh = A_k_cache.shape
        W = min(4096, max(256, Sk // 4))
        F = B_w_gate.shape[1]
        scale = Dh ** -0.5
        S0 = Sk - W
        G = 8
        NG = H // G
        TK = 128
        HK = TK // 2
        NJ = W // TK
        GD = G * Dh
        NE = 2 * NJ
        OP = GD // NE
        QP = D // NE
        F1 = NE * OP
        f32 = jnp.float32
        bf16 = jnp.bfloat16

        def kernel(x_hbm, k_hbm, v_hbm, wq_hbm, wo_hbm, wg_hbm, wu_hbm, wd_hbm, gw_hbm, o_hbm,
                   x_v, gw_v, ring, wqbuf, wobuf, wgbuf, wubuf, wdbuf, o_v, s_scr, hid_v, out_v,
                   sem_misc, sem_b, sem_w):
            def al(i, n):
                return i if isinstance(i, int) else pl.multiple_of(i, n)

            def bulk(src, g, j, slot, i):
                return pltpu.make_async_copy(
                    src.at[0, pl.ds(g * G, G), pl.ds(al(S0 + j * TK + i * HK, HK), HK), :],
                    ring.at[slot, :, pl.ds(i * HK, HK), :], sem_b.at[slot * 2 + i])

            def bulk_wait(slot, i):
                dst = ring.at[slot, :, pl.ds(i * HK, HK), :]
                pltpu.make_async_copy(dst, dst, sem_b.at[slot * 2 + i]).wait()

            def wq_piece(g, e, n=QP):
                return pltpu.make_async_copy(
                    wq_hbm.at[pl.ds(al(e * n, n), n), pl.ds(al(g * GD, GD), GD)],
                    wqbuf.at[pl.ds(al(e * n, n), n), :], sem_w.at[0])

            def wo_piece(g, e):
                return pltpu.make_async_copy(
                    wo_hbm.at[pl.ds(al(g * GD + e * OP, OP), OP), :],
                    wobuf.at[pl.ds(al(e * OP, OP), OP), :], sem_w.at[1])

            def wd_copy(r0, n, sem):
                return pltpu.make_async_copy(wd_hbm.at[pl.ds(r0, n), :], wdbuf.at[pl.ds(r0, n), :], sem)

            def wait_all(ref, sem):
                pltpu.make_async_copy(ref, ref, sem).wait()

            cp_x = pltpu.make_async_copy(x_hbm, x_v, sem_misc.at[0])
            cp_gw = pltpu.make_async_copy(gw_hbm, gw_v, sem_misc.at[1])
            cp_wg = pltpu.make_async_copy(wg_hbm, wgbuf, sem_misc.at[2])
            cp_wu = pltpu.make_async_copy(wu_hbm, wubuf, sem_misc.at[3])
            cp_wd3 = wd_copy(F1, F - F1, sem_misc.at[5])

            cp_wg.start(priority=PB)
            cp_x.start(priority=PT)
            cp_gw.start(priority=PT)
            cp_wu.start(priority=PB)
            wq_piece(0, 0, D).start(priority=PB)
            cp_x.wait()
            x = x_v[0]
            x8 = jnp.broadcast_to(x, (8, D))
            cp_gw.wait()
            for n in range(NB):
                for i in range(2):
                    bulk(k_hbm, 0, n, n, i).start(priority=PB)
            gw = gw_v[...].reshape(1, D).astype(f32)
            gate = jax.nn.sigmoid(jnp.sum(x.astype(f32) * gw, axis=-1, keepdims=True))
            out_v[...] = jnp.zeros_like(out_v)
            cp_wg.wait()
            gt = lax.dot_general(x8, wgbuf[...], NT, preferred_element_type=f32)
            cp_wu.wait()
            u = lax.dot_general(x8, wubuf[...], NT, preferred_element_type=f32)
            hid_v[...] = (gt * jax.nn.sigmoid(gt) * u).astype(bf16)
            bulk_wait(0, 0)

            row = lax.broadcasted_iota(jnp.int32, (G, GD), 0)
            colh = lax.broadcasted_iota(jnp.int32, (G, GD), 1) // Dh
            diag = row == colh

            def group(g, _):
                wait_all(wqbuf, sem_w.at[0])
                q = jnp.dot(x8, wqbuf[...], preferred_element_type=f32)
                qbd = jnp.where(diag, q, 0.0).astype(bf16)

                def prefetch(phase, j, i):
                    jn = j + NB
                    slot = jn % R

                    @pl.when(jn < NJ)
                    def _():
                        bulk(v_hbm if phase else k_hbm, g, jn, slot, i).start(priority=PB)

                    if phase == 0:
                        @pl.when(jn >= NJ)
                        def _():
                            bulk(v_hbm, g, jn - NJ, slot, i).start(priority=PB)
                    else:
                        @pl.when(jnp.logical_and(jn >= NJ, g + 1 < NG))
                        def _():
                            bulk(k_hbm, g + 1, jn - NJ, slot, i).start(priority=PB)
                        if i == 0:
                            @pl.when(jnp.logical_and(jn == NJ, g + 1 == NG))
                            def _():
                                cp_wd3.start(priority=PB)

                def trickle(phase, e):
                    if phase == 0:
                        wo_piece(g, e).start(priority=PT)
                    else:
                        @pl.when(g + 1 < NG)
                        def _():
                            wq_piece(g + 1, e).start(priority=PT)

                        @pl.when(g + 1 == NG)
                        def _():
                            wd_copy(al(e * OP, OP), OP, sem_misc.at[4]).start(priority=PT)

                def tick_start(phase, j):
                    bulk_wait(j % R, 1)
                    trickle(phase, 2 * j)
                    prefetch(phase, j, 0)
                    if not STAG:
                        prefetch(phase, j, 1)

                def tick_mid(phase, j):
                    if phase == 0:
                        bulk_wait((j + 1) % R, 0)
                    else:
                        @pl.when(jnp.logical_or(j + 1 < NJ, g + 1 < NG))
                        def _():
                            bulk_wait((j + 1) % R, 0)
                    trickle(phase, 2 * j + 1)
                    if STAG:
                        prefetch(phase, j, 1)

                def kbody(j, _):
                    tick_start(0, j)
                    slot = j % R
                    s = None
                    for h in range(G):
                        d = lax.dot_general(qbd[:, h * Dh:(h + 1) * Dh], ring[slot, h], NT,
                                            preferred_element_type=f32)
                        s = d if s is None else s + d
                    s_scr[j] = s
                    tick_mid(0, j)
                    return 0

                lax.fori_loop(0, NJ, kbody, 0)

                s = s_scr[...] * scale
                m = jnp.max(jnp.max(s, axis=0), axis=-1, keepdims=True)
                p = jnp.exp(s - m[None])
                l = jnp.sum(jnp.sum(p, axis=0), axis=-1, keepdims=True)
                s_scr[...] = p

                def vbody(j, accs):
                    tick_start(1, j)
                    slot = j % R
                    pj = s_scr[j].astype(bf16)
                    accs = tuple(
                        accs[h] + jnp.dot(pj, ring[slot, h], preferred_element_type=f32)
                        for h in range(G))
                    tick_mid(1, j)
                    return accs

                accs = lax.fori_loop(0, NJ, vbody, tuple(jnp.zeros((G, Dh), f32) for _ in range(G)))
                o = jnp.concatenate(accs, axis=1) / l
                obd = jnp.where(diag, o, 0.0).astype(bf16)
                wait_all(wobuf, sem_w.at[1])
                out_v[...] += jnp.dot(obd, wobuf[...], preferred_element_type=f32)
                return 0

            lax.fori_loop(0, NG, group, 0)

            a = jnp.sum(out_v[...], axis=0, keepdims=True)
            wd_copy(0, F1, sem_misc.at[4]).wait()
            cp_wd3.wait()
            b = jnp.dot(hid_v[...], wdbuf[...], preferred_element_type=f32)
            res = gate * a + (1.0 - gate) * b[0:1]
            o_v[0] = res.astype(o_v.dtype)
            cp_o = pltpu.make_async_copy(o_v, o_hbm, sem_misc.at[6])
            cp_o.start()
            cp_o.wait()

        any_spec = pl.BlockSpec(memory_space=pl.ANY)
        return pl.pallas_call(
            kernel,
            in_specs=[any_spec] * 9,
            out_specs=any_spec,
            out_shape=jax.ShapeDtypeStruct((B, Sq, D), A_x.dtype),
            scratch_shapes=[
                pltpu.VMEM((1, 1, D), bf16), pltpu.VMEM((D,), bf16),
                pltpu.VMEM((R, G, TK, Dh), bf16),
                pltpu.VMEM((D, GD), bf16), pltpu.VMEM((GD, D), bf16),
                pltpu.VMEM((F, D), bf16), pltpu.VMEM((F, D), bf16), pltpu.VMEM((F, D), bf16),
                pltpu.VMEM((1, 1, D), bf16), pltpu.VMEM((NJ, G, TK), f32), pltpu.VMEM((8, F), bf16),
                pltpu.VMEM((G, D), f32),
                pltpu.SemaphoreType.DMA((7,)), pltpu.SemaphoreType.DMA((2 * R,)),
                pltpu.SemaphoreType.DMA((2,)),
            ],
            compiler_params=pltpu.CompilerParams(vmem_limit_bytes=64 * 1024 * 1024,
                                                 disable_bounds_checks=cfg["NOBC"],
                                                 disable_semaphore_checks=cfg["NOSC"]),
        )(A_x, A_k_cache, A_v_cache, A_wq, A_wo, B_w_gate.T, B_w_up.T, B_w_down, gate_w)

    return jax.jit(fn)


pallas_gated_mix__sliding_block_cached__swiglu_ffn__decode_kernel = build(CFG)
```

```python
import functools
import jax
import jax.numpy as jnp
from jax import lax
import jax.experimental.pallas as pl
import jax.experimental.pallas.tpu as pltpu

CFG = dict(R=8, NB=6, NOBC=True, NOSC=True, STAG=False, L0=48)

NT = (((1,), (1,)), ((), ()))
PT, PB = 0, 1


def build(cfg):
    R = cfg["R"]; NB = cfg["NB"]; STAG = cfg["STAG"]

    def fn(A_x, A_k_cache, A_v_cache, A_wq, A_wo, B_x, B_w_gate, B_w_up, B_w_down, gate_w):
        B, Sq, D = A_x.shape
        _, H, Sk, Dh = A_k_cache.shape
        W = min(4096, max(256, Sk // 4))
        F = B_w_gate.shape[1]
        scale = Dh ** -0.5
        S0 = Sk - W
        G = 8
        NG = H // G
        TK = 128
        LEN = (cfg["L0"], TK - cfg["L0"])
        OFF = (0, cfg["L0"])
        NJ = W // TK
        GD = G * Dh
        NE = 2 * NJ
        OP = GD // NE
        QP = D // NE
        F1 = NE * OP
        f32 = jnp.float32
        bf16 = jnp.bfloat16

        def kernel(x_hbm, k_hbm, v_hbm, wq_hbm, wo_hbm, wg_hbm, wu_hbm, wd_hbm, gw_hbm, o_hbm,
                   x_v, gw_v, ring, wqbuf, wobuf, wgbuf, wubuf, wdbuf, o_v, s_scr, hid_v, out_v,
                   sem_misc, sem_b, sem_w):
            def al(i, n):
                return i if isinstance(i, int) else pl.multiple_of(i, n)

            def bulk(src, g, j, slot, i):
                return pltpu.make_async_copy(
                    src.at[0, pl.ds(g * G, G), pl.ds(al(S0 + j * TK + OFF[i], 8), LEN[i]), :],
                    ring.at[slot, :, pl.ds(OFF[i], LEN[i]), :], sem_b.at[slot * 2 + i])

            def bulk_wait(slot, i):
                dst = ring.at[slot, :, pl.ds(OFF[i], LEN[i]), :]
                pltpu.make_async_copy(dst, dst, sem_b.at[slot * 2 + i]).wait()

            def wq_piece(g, e, n=QP):
                return pltpu.make_async_copy(
                    wq_hbm.at[pl.ds(al(e * n, n), n), pl.ds(al(g * GD, GD), GD)],
                    wqbuf.at[pl.ds(al(e * n, n), n), :], sem_w.at[0])

            def wo_piece(g, e):
                return pltpu.make_async_copy(
                    wo_hbm.at[pl.ds(al(g * GD + e * OP, OP), OP), :],
                    wobuf.at[pl.ds(al(e * OP, OP), OP), :], sem_w.at[1])

            def wd_copy(r0, n, sem):
                return pltpu.make_async_copy(wd_hbm.at[pl.ds(r0, n), :], wdbuf.at[pl.ds(r0, n), :], sem)

            def wait_all(ref, sem):
                pltpu.make_async_copy(ref, ref, sem).wait()

            cp_x = pltpu.make_async_copy(x_hbm, x_v, sem_misc.at[0])
            cp_gw = pltpu.make_async_copy(gw_hbm, gw_v, sem_misc.at[1])
            cp_wg = pltpu.make_async_copy(wg_hbm, wgbuf, sem_misc.at[2])
            cp_wu = pltpu.make_async_copy(wu_hbm, wubuf, sem_misc.at[3])
            cp_wd3 = wd_copy(F1, F - F1, sem_misc.at[5])

            cp_wg.start(priority=PB)
            cp_x.start(priority=PT)
            cp_gw.start(priority=PT)
            cp_wu.start(priority=PB)
            wq_piece(0, 0, D).start(priority=PB)
            cp_x.wait()
            x = x_v[0]
            x8 = jnp.broadcast_to(x, (8, D))
            cp_gw.wait()
            for n in range(NB):
                for i in range(2):
                    bulk(k_hbm, 0, n, n, i).start(priority=PB)
            gw = gw_v[...].reshape(1, D).astype(f32)
            gate = jax.nn.sigmoid(jnp.sum(x.astype(f32) * gw, axis=-1, keepdims=True))
            out_v[...] = jnp.zeros_like(out_v)
            cp_wg.wait()
            gt = lax.dot_general(x8, wgbuf[...], NT, preferred_element_type=f32)
            cp_wu.wait()
            u = lax.dot_general(x8, wubuf[...], NT, preferred_element_type=f32)
            hid_v[...] = (gt * jax.nn.sigmoid(gt) * u).astype(bf16)
            bulk_wait(0, 0)

            row = lax.broadcasted_iota(jnp.int32, (G, GD), 0)
            colh = lax.broadcasted_iota(jnp.int32, (G, GD), 1) // Dh
            diag = row == colh

            def group(g, _):
                wait_all(wqbuf, sem_w.at[0])
                q = jnp.dot(x8, wqbuf[...], preferred_element_type=f32)
                qbd = jnp.where(diag, q, 0.0).astype(bf16)

                def prefetch(phase, j, i):
                    jn = j + NB
                    slot = jn % R

                    @pl.when(jn < NJ)
                    def _():
                        bulk(v_hbm if phase else k_hbm, g, jn, slot, i).start(priority=PB)

                    if phase == 0:
                        @pl.when(jn >= NJ)
                        def _():
                            bulk(v_hbm, g, jn - NJ, slot, i).start(priority=PB)
                    else:
                        @pl.when(jnp.logical_and(jn >= NJ, g + 1 < NG))
                        def _():
                            bulk(k_hbm, g + 1, jn - NJ, slot, i).start(priority=PB)
                        if i == 0:
                            @pl.when(jnp.logical_and(jn == NJ, g + 1 == NG))
                            def _():
                                cp_wd3.start(priority=PB)

                def trickle(phase, e):
                    if phase == 0:
                        wo_piece(g, e).start(priority=PT)
                    else:
                        @pl.when(g + 1 < NG)
                        def _():
                            wq_piece(g + 1, e).start(priority=PT)

                        @pl.when(g + 1 == NG)
                        def _():
                            wd_copy(al(e * OP, OP), OP, sem_misc.at[4]).start(priority=PT)

                def tick_start(phase, j):
                    bulk_wait(j % R, 1)
                    trickle(phase, 2 * j)
                    prefetch(phase, j, 0)
                    if not STAG:
                        prefetch(phase, j, 1)

                def tick_mid(phase, j):
                    if phase == 0:
                        bulk_wait((j + 1) % R, 0)
                    else:
                        @pl.when(jnp.logical_or(j + 1 < NJ, g + 1 < NG))
                        def _():
                            bulk_wait((j + 1) % R, 0)
                    trickle(phase, 2 * j + 1)
                    if STAG:
                        prefetch(phase, j, 1)

                def kbody(j, _):
                    tick_start(0, j)
                    slot = j % R
                    s = None
                    for h in range(G):
                        d = lax.dot_general(qbd[:, h * Dh:(h + 1) * Dh], ring[slot, h], NT,
                                            preferred_element_type=f32)
                        s = d if s is None else s + d
                    s_scr[j] = s
                    tick_mid(0, j)
                    return 0

                lax.fori_loop(0, NJ, kbody, 0)

                s = s_scr[...] * scale
                m = jnp.max(jnp.max(s, axis=0), axis=-1, keepdims=True)
                p = jnp.exp(s - m[None])
                l = jnp.sum(jnp.sum(p, axis=0), axis=-1, keepdims=True)
                s_scr[...] = p

                def vbody(j, accs):
                    tick_start(1, j)
                    slot = j % R
                    pj = s_scr[j].astype(bf16)
                    accs = tuple(
                        accs[h] + jnp.dot(pj, ring[slot, h], preferred_element_type=f32)
                        for h in range(G))
                    tick_mid(1, j)
                    return accs

                accs = lax.fori_loop(0, NJ, vbody, tuple(jnp.zeros((G, Dh), f32) for _ in range(G)))
                o = jnp.concatenate(accs, axis=1) / l
                obd = jnp.where(diag, o, 0.0).astype(bf16)
                wait_all(wobuf, sem_w.at[1])
                out_v[...] += jnp.dot(obd, wobuf[...], preferred_element_type=f32)
                return 0

            lax.fori_loop(0, NG, group, 0)

            a = jnp.sum(out_v[...], axis=0, keepdims=True)
            wd_copy(0, F1, sem_misc.at[4]).wait()
            cp_wd3.wait()
            b = jnp.dot(hid_v[...], wdbuf[...], preferred_element_type=f32)
            res = gate * a + (1.0 - gate) * b[0:1]
            o_v[0] = res.astype(o_v.dtype)
            cp_o = pltpu.make_async_copy(o_v, o_hbm, sem_misc.at[6])
            cp_o.start()
            cp_o.wait()

        any_spec = pl.BlockSpec(memory_space=pl.ANY)
        return pl.pallas_call(
            kernel,
            in_specs=[any_spec] * 9,
            out_specs=any_spec,
            out_shape=jax.ShapeDtypeStruct((B, Sq, D), A_x.dtype),
            scratch_shapes=[
                pltpu.VMEM((1, 1, D), bf16), pltpu.VMEM((D,), bf16),
                pltpu.VMEM((R, G, TK, Dh), bf16),
                pltpu.VMEM((D, GD), bf16), pltpu.VMEM((GD, D), bf16),
                pltpu.VMEM((F, D), bf16), pltpu.VMEM((F, D), bf16), pltpu.VMEM((F, D), bf16),
                pltpu.VMEM((1, 1, D), bf16), pltpu.VMEM((NJ, G, TK), f32), pltpu.VMEM((8, F), bf16),
                pltpu.VMEM((G, D), f32),
                pltpu.SemaphoreType.DMA((7,)), pltpu.SemaphoreType.DMA((2 * R,)),
                pltpu.SemaphoreType.DMA((2,)),
            ],
            compiler_params=pltpu.CompilerParams(vmem_limit_bytes=64 * 1024 * 1024,
                                                 disable_bounds_checks=cfg["NOBC"],
                                                 disable_semaphore_checks=cfg["NOSC"]),
        )(A_x, A_k_cache, A_v_cache, A_wq, A_wo, B_w_gate.T, B_w_up.T, B_w_down, gate_w)

    return jax.jit(fn)


pallas_gated_mix__sliding_block_cached__swiglu_ffn__decode_kernel = build(CFG)
```

```python
import functools
import jax
import jax.numpy as jnp
from jax import lax
import jax.experimental.pallas as pl
import jax.experimental.pallas.tpu as pltpu

CFG = dict(R=8, NB=6, NOBC=True, NOSC=True, L0=80, LO=8, JQ=4, JB=27, JG=8, JU=8, P1=40, F1=1024, E3=True)

NT = (((1,), (1,)), ((), ()))
PT, PB = 0, 1


def build(cfg):
    R = cfg["R"]; NB = cfg["NB"]; LO = cfg["LO"]; JQ = cfg["JQ"]; JB = cfg["JB"]
    JG = cfg["JG"]; JU = cfg["JU"]; P1 = cfg["P1"]; E3 = cfg["E3"]

    def fn(A_x, A_k_cache, A_v_cache, A_wq, A_wo, B_x, B_w_gate, B_w_up, B_w_down, gate_w):
        B, Sq, D = A_x.shape
        _, H, Sk, Dh = A_k_cache.shape
        W = min(4096, max(256, Sk // 4))
        F = B_w_gate.shape[1]
        scale = Dh ** -0.5
        S0 = Sk - W
        G = 8
        NG = H // G
        TK = 128
        LEN = (cfg["L0"], TK - cfg["L0"])
        OFF = (0, cfg["L0"])
        NJ = W // TK
        GD = G * Dh
        NTICK = NG * 2 * NJ
        OP = H * Dh // NTICK
        QP = D // (2 * NJ)
        FP = 16
        NFP = F // FP
        assert NFP * FP == F and NFP <= (NG - 1) * NJ
        DP = 8
        F1 = cfg["F1"]
        NDP = F1 // DP
        ND0 = 2 * ((NG - 1) * NJ - NFP)
        f32 = jnp.float32
        bf16 = jnp.bfloat16

        def kernel(x_hbm, k_hbm, v_hbm, wq_hbm, wo_hbm, wg_hbm, wu_hbm, wd_hbm, gw_hbm, o_hbm,
                   x_v, gw_v, ring, wqbuf, wobuf, wgbuf, wubuf, wdbuf, o_v, s_scr, q_v, act_v, hid_v, out_v, b_v,
                   sem_misc, sem_b, sem_wo):
            def al(i, n):
                return i if isinstance(i, int) else pl.multiple_of(i, n)

            def bulk(src, g, j, slot, i):
                return pltpu.make_async_copy(
                    src.at[0, pl.ds(g * G, G), pl.ds(al(S0 + j * TK + OFF[i], 8), LEN[i]), :],
                    ring.at[slot, :, pl.ds(OFF[i], LEN[i]), :], sem_b.at[slot * 2 + i])

            def bulk_wait(slot, i, n):
                dst = ring.at[slot, :, pl.ds(OFF[i], n), :]
                pltpu.make_async_copy(dst, dst, sem_b.at[slot * 2 + i]).wait()

            def rows_copy(src, dst, r0, n, sem):
                return pltpu.make_async_copy(src.at[pl.ds(r0, n), :], dst.at[pl.ds(r0, n), :], sem)

            def wq_piece(g, e, n=QP):
                return pltpu.make_async_copy(
                    wq_hbm.at[pl.ds(al(e * n, n), n), pl.ds(al(g * GD, GD), GD)],
                    wqbuf.at[pl.ds(al(e * n, n), n), :], sem_misc.at[2])

            def wo_piece(i):
                return rows_copy(wo_hbm, wobuf, al(i * OP, OP), OP, sem_wo.at[i // (2 * NJ)])

            def wait_ref(ref, sem):
                pltpu.make_async_copy(ref, ref, sem).wait()

            cp_x = pltpu.make_async_copy(x_hbm, x_v, sem_misc.at[0])
            cp_gw = pltpu.make_async_copy(gw_hbm, gw_v, sem_misc.at[1])
            cp_wd3 = rows_copy(wd_hbm, wdbuf, F1, F - F1, sem_misc.at[6])

            row = lax.broadcasted_iota(jnp.int32, (G, GD), 0)
            colh = lax.broadcasted_iota(jnp.int32, (G, GD), 1) // Dh
            diag = row == colh

            wq_piece(0, 0, D).start(priority=PB)
            cp_x.start(priority=PT)
            cp_gw.start(priority=PT)
            out_v[...] = jnp.zeros_like(out_v)
            cp_x.wait()
            cp_gw.wait()
            for n in range(NB):
                for i in range(2):
                    bulk(k_hbm, 0, n, n, i).start(priority=PB)
            for i in range(LO):
                wo_piece(i).start(priority=PT)
                wait_ref(wqbuf.at[pl.ds(0, D // LO), :], sem_misc.at[2])
            x = x_v[0]
            x8 = jnp.broadcast_to(x, (8, D))
            gw = gw_v[...].reshape(1, D).astype(f32)
            gate = jax.nn.sigmoid(jnp.sum(x.astype(f32) * gw, axis=-1, keepdims=True))

            def make_q():
                q = jnp.dot(x8, wqbuf[...], preferred_element_type=f32)
                q_v[...] = jnp.where(diag, q, 0.0)

            make_q()
            bulk_wait(0, 0, LEN[0])
            bulk_wait(0, 1, P1)

            def group(g, _):
                qbd = q_v[...].astype(bf16)
                lastg = g + 1 == NG

                def prefetch(phase, j, i):
                    jn = j + NB
                    slot = jn % R

                    @pl.when(jn < NJ)
                    def _():
                        bulk(v_hbm if phase else k_hbm, g, jn, slot, i).start(priority=PB)

                    if phase == 0:
                        @pl.when(jn >= NJ)
                        def _():
                            bulk(v_hbm, g, jn - NJ, slot, i).start(priority=PB)
                    else:
                        @pl.when(jnp.logical_and(jn >= NJ, g + 1 < NG))
                        def _():
                            bulk(k_hbm, g + 1, jn - NJ, slot, i).start(priority=PB)
                        if i == 0:
                            @pl.when(jnp.logical_and(jn == NJ, lastg))
                            def _():
                                cp_wd3.start(priority=PB)

                def wd_piece(cond, d):
                    @pl.when(cond)
                    def _():
                        rows_copy(wd_hbm, wdbuf, al(d * DP, DP), DP, sem_misc.at[5]).start(priority=PT)

                def tick_start(phase, j):
                    bulk_wait(j % R, 1, LEN[1] - P1)
                    i = (2 * g + phase) * NJ + j + LO
                    if phase == 0:
                        wo_piece(i).start(priority=PT)
                    else:
                        @pl.when(i < NTICK)
                        def _():
                            wo_piece(i).start(priority=PT)
                    prefetch(phase, j, 0)
                    prefetch(phase, j, 1)

                def tick_mid(phase, j, k):
                    n = LEN[0] if k == 0 else P1
                    if phase == 0:
                        if E3 or k == 0:
                            bulk_wait((j + 1) % R, k, n)

                        @pl.when(g + 1 < NG)
                        def _():
                            wq_piece(g + 1, 2 * j + k).start(priority=PT)
                        wd_piece(lastg, ND0 + 2 * j + k)
                        if not E3 and k == 1:
                            bulk_wait((j + 1) % R, k, n)
                    else:
                        def w():
                            @pl.when(jnp.logical_or(j + 1 < NJ, g + 1 < NG))
                            def _():
                                bulk_wait((j + 1) % R, k, n)
                        if E3 or k == 0:
                            w()
                        p = g * NJ + j

                        @pl.when(p < NFP)
                        def _():
                            if k == 0:
                                rows_copy(wg_hbm, wgbuf, al(p * FP, FP), FP, sem_misc.at[3]).start(priority=PT)
                            else:
                                rows_copy(wu_hbm, wubuf, al(p * FP, FP), FP, sem_misc.at[4]).start(priority=PT)
                        d = jnp.where(lastg, ND0 + 2 * NJ + 2 * j + k, 2 * (p - NFP) + k)
                        wd_piece(jnp.logical_and(d >= 0, d < NDP), d)
                        if not E3 and k == 1:
                            w()

                def kbody(j, _):
                    tick_start(0, j)
                    slot = j % R
                    s = None
                    for h in range(G):
                        d = lax.dot_general(qbd[:, h * Dh:(h + 1) * Dh], ring[slot, h], NT,
                                            preferred_element_type=f32)
                        s = d if s is None else s + d
                    s_scr[j] = s
                    tick_mid(0, j, 0)

                    @pl.when(jnp.logical_and(lastg, j == JG))
                    def _():
                        wait_ref(wgbuf, sem_misc.at[3])
                        gt = lax.dot_general(x8, wgbuf[...], NT, preferred_element_type=f32)
                        act_v[...] = gt * jax.nn.sigmoid(gt)

                    @pl.when(jnp.logical_and(lastg, j == JG + JU))
                    def _():
                        wait_ref(wubuf, sem_misc.at[4])
                        u = lax.dot_general(x8, wubuf[...], NT, preferred_element_type=f32)
                        hid_v[...] = (act_v[...] * u).astype(bf16)
                    tick_mid(0, j, 1)
                    return 0

                lax.fori_loop(0, NJ, kbody, 0)

                s = s_scr[...] * scale
                m = jnp.max(jnp.max(s, axis=0), axis=-1, keepdims=True)
                p = jnp.exp(s - m[None])
                l = jnp.sum(jnp.sum(p, axis=0), axis=-1, keepdims=True)
                s_scr[...] = p

                def vbody(j, accs):
                    tick_start(1, j)
                    slot = j % R
                    pj = s_scr[j].astype(bf16)
                    accs = tuple(
                        accs[h] + jnp.dot(pj, ring[slot, h], preferred_element_type=f32)
                        for h in range(G))
                    tick_mid(1, j, 0)

                    @pl.when(jnp.logical_and(g + 1 < NG, j == JQ))
                    def _():
                        wait_ref(wqbuf, sem_misc.at[2])
                        make_q()

                    @pl.when(jnp.logical_and(lastg, j == JB))
                    def _():
                        wait_ref(wdbuf.at[pl.ds(0, F1), :], sem_misc.at[5])
                        b_v[...] = jnp.dot(hid_v[:, :F1], wdbuf[pl.ds(0, F1), :], preferred_element_type=f32)
                    tick_mid(1, j, 1)
                    return accs

                accs = lax.fori_loop(0, NJ, vbody, tuple(jnp.zeros((G, Dh), f32) for _ in range(G)))
                o = jnp.concatenate(accs, axis=1) / l
                obd = jnp.where(diag, o, 0.0).astype(bf16)
                wo_g = wobuf.at[pl.ds(al(g * GD, GD), GD), :]
                wait_ref(wo_g, sem_wo.at[g])
                out_v[...] += jnp.dot(obd, wo_g[...], preferred_element_type=f32)
                return 0

            lax.fori_loop(0, NG, group, 0)

            part = gate * jnp.sum(out_v[...], axis=0, keepdims=True) + (1.0 - gate) * b_v[0:1, :]
            cp_wd3.wait()
            b = jnp.dot(hid_v[:, F1:], wdbuf[pl.ds(F1, F - F1), :], preferred_element_type=f32)
            res = part + (1.0 - gate) * b[0:1]
            o_v[0] = res.astype(o_v.dtype)
            cp_o = pltpu.make_async_copy(o_v, o_hbm, sem_misc.at[7])
            cp_o.start()
            cp_o.wait()

        any_spec = pl.BlockSpec(memory_space=pl.ANY)
        return pl.pallas_call(
            kernel,
            in_specs=[any_spec] * 9,
            out_specs=any_spec,
            out_shape=jax.ShapeDtypeStruct((B, Sq, D), A_x.dtype),
            scratch_shapes=[
                pltpu.VMEM((1, 1, D), bf16), pltpu.VMEM((D,), bf16),
                pltpu.VMEM((R, G, TK, Dh), bf16),
                pltpu.VMEM((D, GD), bf16), pltpu.VMEM((H * Dh, D), bf16),
                pltpu.VMEM((F, D), bf16), pltpu.VMEM((F, D), bf16), pltpu.VMEM((F, D), bf16),
                pltpu.VMEM((1, 1, D), bf16), pltpu.VMEM((NJ, G, TK), f32), pltpu.VMEM((G, GD), f32),
                pltpu.VMEM((8, F), f32), pltpu.VMEM((8, F), bf16),
                pltpu.VMEM((G, D), f32), pltpu.VMEM((8, D), f32),
                pltpu.SemaphoreType.DMA((8,)), pltpu.SemaphoreType.DMA((2 * R,)),
                pltpu.SemaphoreType.DMA((NG,)),
            ],
            compiler_params=pltpu.CompilerParams(vmem_limit_bytes=64 * 1024 * 1024,
                                                 disable_bounds_checks=cfg["NOBC"],
                                                 disable_semaphore_checks=cfg["NOSC"]),
        )(A_x, A_k_cache, A_v_cache, A_wq, A_wo, B_w_gate.T, B_w_up.T, B_w_down, gate_w)

    return jax.jit(fn)


pallas_gated_mix__sliding_block_cached__swiglu_ffn__decode_kernel = build(CFG)
```

```python
import jax
import jax.numpy as jnp
from jax import lax
import jax.experimental.pallas as pl
import jax.experimental.pallas.tpu as pltpu

_NT = (((1,), (1,)), ((), ()))
_PT, _PB = 0, 1

_G = 8
_TK = 128
_R = 8
_NB = 5
_ROWS = (40, 72, 16)
_LO = 8
_JQ, _JG, _JU, _JB = 4, 8, 16, 27
_FV, _FM = 128, 384


def _compiler_params():
    kwargs = dict(vmem_limit_bytes=64 * 1024 * 1024)
    for name in ("disable_bounds_checks", "disable_semaphore_checks"):
        if hasattr(pltpu.CompilerParams, name):
            kwargs[name] = True
    return pltpu.CompilerParams(**kwargs)


@jax.jit
def pallas_gated_mix__sliding_block_cached__swiglu_ffn__decode_kernel(
    A_x: jax.Array,
    A_k_cache: jax.Array,
    A_v_cache: jax.Array,
    A_wq: jax.Array,
    A_wo: jax.Array,
    B_x: jax.Array,
    B_w_gate: jax.Array,
    B_w_up: jax.Array,
    B_w_down: jax.Array,
    gate_w: jax.Array,
):
    del B_x
    B, Sq, D = A_x.shape
    _, H, Sk, Dh = A_k_cache.shape
    F = B_w_gate.shape[1]
    W = min(4096, max(256, Sk // 4))
    S0 = Sk - W
    scale = Dh ** -0.5
    f32, bf16 = jnp.float32, jnp.bfloat16

    G, TK, R, NB, LO, FV, FM = _G, _TK, _R, _NB, _LO, _FV, _FM
    NG = H // G
    NJ = W // TK
    GD = G * Dh
    NTICK = 2 * NG * NJ
    NP = len(_ROWS)
    ROW0 = tuple(sum(_ROWS[:i]) for i in range(NP))
    OP = H * Dh // NTICK
    QP = D // (2 * NJ)
    FP = 16
    NFP = F // FP
    DP = 8
    F1 = FV + FM
    NDP = (F - F1) // DP
    assert B == 1 and Sq == 1 and A_wq.shape == (D, H * Dh) and Dh == 128 and D % 128 == 0
    assert H % G == 0 and NG >= 2 and W % TK == 0 and S0 % 8 == 0 and sum(_ROWS) == TK
    assert NB < R and NJ % R == 0 and NB <= LO and NB + 1 <= NJ and D % (8 * LO) == 0
    assert OP % 8 == 0 and OP * NTICK == H * Dh and QP % 8 == 0 and QP * 2 * NJ == D
    assert NFP * FP == F and NFP <= (NG - 1) * NJ
    assert FV == 128 and F1 % 128 == 0 and NDP * DP == F - F1
    assert 2 * NJ <= NDP <= 2 * (NJ + _JB - 2) and _JG < _JU < NJ and _JB < NJ and _JQ < NJ

    def kernel(x_hbm, k_hbm, v_hbm, wq_hbm, wo_hbm, wg_hbm, wu_hbm, wd_hbm, gw_hbm, o_hbm,
               x_v, gw_v, ring, wqbuf, wobuf, wgbuf, wubuf, wdbuf, o_v,
               s_scr, q_v, act_v, hid_v, hcol_v, out_v, b_v, sem, sem_kv, sem_wo):
        def al(i, n):
            return i if isinstance(i, int) else pl.multiple_of(i, n)

        def kv_copy(src, g, j, slot, i):
            return pltpu.make_async_copy(
                src.at[0, pl.ds(g * G, G), pl.ds(al(S0 + j * TK + ROW0[i], 8), _ROWS[i]), :],
                ring.at[slot, :, pl.ds(ROW0[i], _ROWS[i]), :], sem_kv.at[slot * NP + i])

        def wait_ref(ref, s):
            pltpu.make_async_copy(ref, ref, s).wait()

        def kv_wait(slot, i):
            wait_ref(ring.at[slot, :, pl.ds(ROW0[i], _ROWS[i]), :], sem_kv.at[slot * NP + i])

        def rows_copy(src, dst, r0, n, s):
            return pltpu.make_async_copy(src.at[pl.ds(r0, n), :], dst.at[pl.ds(r0, n), :], s)

        def wq_piece(g, e, n=QP):
            return pltpu.make_async_copy(
                wq_hbm.at[pl.ds(al(e * n, n), n), pl.ds(al(g * GD, GD), GD)],
                wqbuf.at[pl.ds(al(e * n, n), n), :], sem.at[2])

        def wo_piece(i):
            return rows_copy(wo_hbm, wobuf, al(i * OP, OP), OP, sem_wo.at[i // (2 * NJ)])

        cp_x = pltpu.make_async_copy(x_hbm, x_v, sem.at[0])
        cp_gw = pltpu.make_async_copy(gw_hbm, gw_v, sem.at[1])
        cp_wdm = rows_copy(wd_hbm, wdbuf, FV, FM, sem.at[6])
        cp_wdv = rows_copy(wd_hbm, wdbuf, 0, FV, sem.at[7])

        diag = (lax.broadcasted_iota(jnp.int32, (G, GD), 0)
                == lax.broadcasted_iota(jnp.int32, (G, GD), 1) // Dh)

        for i in range(LO):
            wq_piece(0, i, D // LO).start(priority=_PB)
        cp_x.start(priority=_PT)
        cp_gw.start(priority=_PT)
        out_v[...] = jnp.zeros_like(out_v)
        cp_x.wait()
        cp_gw.wait()
        for i in range(LO):
            wo_piece(i).start(priority=_PT)
            if i < NB:
                for k in range(NP):
                    kv_copy(k_hbm, 0, i, i, k).start(priority=_PB)
            wq_piece(0, i, D // LO).wait()
        x = x_v[0]
        x8 = jnp.broadcast_to(x, (8, D))
        gw = gw_v[...].reshape(1, D).astype(f32)
        gate = jax.nn.sigmoid(jnp.sum(x.astype(f32) * gw, axis=-1, keepdims=True))

        def make_q():
            q = jnp.dot(x8, wqbuf[...], preferred_element_type=f32)
            q_v[...] = jnp.where(diag, q, 0.0)

        make_q()
        kv_wait(0, 0)
        kv_wait(0, 1)

        def group(g, carry):
            qbd = q_v[...].astype(bf16)
            lastg = g + 1 == NG

            def prefetch(phase, j):
                jn = j + NB
                slot = jn % R

                def start(src, gg, jj):
                    for i in range(NP):
                        kv_copy(src, gg, jj, slot, i).start(priority=_PB)

                @pl.when(jn < NJ)
                def _():
                    start(v_hbm if phase else k_hbm, g, jn)

                if phase == 0:
                    @pl.when(jn >= NJ)
                    def _():
                        start(v_hbm, g, jn - NJ)
                else:
                    @pl.when(jnp.logical_and(jn >= NJ, g + 1 < NG))
                    def _():
                        start(k_hbm, g + 1, jn - NJ)

                    @pl.when(jnp.logical_and(jn == NJ, lastg))
                    def _():
                        cp_wdm.start(priority=_PB)

                    @pl.when(jnp.logical_and(jn == NJ + 1, lastg))
                    def _():
                        cp_wdv.start(priority=_PB)

            def tick_start(phase, j):
                kv_wait(j % R, NP - 1)
                i = (2 * g + phase) * NJ + j + LO

                @pl.when(i < NTICK)
                def _():
                    wo_piece(i).start(priority=_PT)
                prefetch(phase, j)

            def tick_mid(phase, j, k):
                if phase == 0:
                    kv_wait((j + 1) % R, k)

                    @pl.when(g + 1 < NG)
                    def _():
                        wq_piece(g + 1, 2 * j + k).start(priority=_PT)
                else:
                    @pl.when(jnp.logical_or(j + 1 < NJ, g + 1 < NG))
                    def _():
                        kv_wait((j + 1) % R, k)
                    p = g * NJ + j
                    src, dst = ((wg_hbm, wgbuf), (wu_hbm, wubuf))[k]

                    @pl.when(p < NFP)
                    def _():
                        rows_copy(src, dst, al(p * FP, FP), FP, sem.at[3 + k]).start(priority=_PT)
                d = 2 * (phase * NJ + j) + k

                @pl.when(jnp.logical_and(lastg, d < NDP))
                def _():
                    rows_copy(wd_hbm, wdbuf, al(F1 + d * DP, DP), DP, sem.at[5]).start(priority=_PT)

            def kbody(j, c):
                tick_start(0, j)
                slot = j % R
                s = None
                for h in range(G):
                    d = lax.dot_general(qbd[:, h * Dh:(h + 1) * Dh], ring[slot, h], _NT,
                                        preferred_element_type=f32)
                    s = d if s is None else s + d
                s_scr[j] = s
                tick_mid(0, j, 0)

                @pl.when(jnp.logical_and(lastg, j == _JG))
                def _():
                    wait_ref(wgbuf, sem.at[3])
                    gt = lax.dot_general(x8, wgbuf[...], _NT, preferred_element_type=f32)
                    act_v[...] = gt * jax.nn.sigmoid(gt)

                @pl.when(jnp.logical_and(lastg, j == _JU))
                def _():
                    wait_ref(wubuf, sem.at[4])
                    u = lax.dot_general(x8, wubuf[...], _NT, preferred_element_type=f32)
                    hid_v[...] = (act_v[...] * u).astype(bf16)
                tick_mid(0, j, 1)
                return c

            lax.fori_loop(0, NJ, kbody, 0)

            s = s_scr[...] * scale
            m = jnp.max(jnp.max(s, axis=0), axis=-1, keepdims=True)
            p = jnp.exp(s - m[None])
            l = jnp.sum(jnp.sum(p, axis=0), axis=-1, keepdims=True)
            s_scr[...] = p

            def vbody(j, accs):
                tick_start(1, j)
                slot = j % R
                pj = s_scr[j].astype(bf16)
                accs = tuple(accs[h] + jnp.dot(pj, ring[slot, h], preferred_element_type=f32)
                             for h in range(G))
                tick_mid(1, j, 0)

                @pl.when(jnp.logical_and(g + 1 < NG, j == _JQ))
                def _():
                    wait_ref(wqbuf, sem.at[2])
                    make_q()

                @pl.when(jnp.logical_and(lastg, j == _JB))
                def _():
                    wait_ref(wdbuf.at[pl.ds(F1, F - F1), :], sem.at[5])
                    b_v[...] = jnp.dot(hid_v[:, F1:], wdbuf[pl.ds(F1, F - F1), :],
                                       preferred_element_type=f32)
                    h0 = hid_v[0:1, 0:FV].astype(f32) * (1.0 - gate)
                    hcol_v[...] = jnp.broadcast_to(h0, (128, FV)).T
                tick_mid(1, j, 1)
                return accs

            accs = lax.fori_loop(0, NJ, vbody, tuple(jnp.zeros((G, Dh), f32) for _ in range(G)))
            o = jnp.concatenate(accs, axis=1) / l
            obd = jnp.where(diag, o, 0.0).astype(bf16)
            wo_g = wobuf.at[pl.ds(al(g * GD, GD), GD), :]
            wait_ref(wo_g, sem_wo.at[g])
            out_v[...] += jnp.dot(obd, wo_g[...], preferred_element_type=f32)
            return carry

        lax.fori_loop(0, NG, group, 0)

        cp_wdm.wait()
        bm = jnp.dot(hid_v[:, FV:F1], wdbuf[pl.ds(FV, FM), :], preferred_element_type=f32)
        part = gate * out_v[...] + ((1.0 - gate) * 0.125) * (b_v[...] + bm)
        hc = hcol_v[...]
        cp_wdv.wait()
        hc = jnp.concatenate([hc] * (D // 128), axis=1)
        prod = (wdbuf[pl.ds(0, FV), :].astype(f32) * hc).reshape(FV // 8, 8, D)
        res = jnp.sum(part + jnp.sum(prod, axis=0), axis=0, keepdims=True)
        o_v[0] = res.astype(o_v.dtype)
        cp_o = pltpu.make_async_copy(o_v, o_hbm, sem.at[0])
        cp_o.start()
        cp_o.wait()

    any_spec = pl.BlockSpec(memory_space=pl.ANY)
    return pl.pallas_call(
        kernel,
        in_specs=[any_spec] * 9,
        out_specs=any_spec,
        out_shape=jax.ShapeDtypeStruct((B, Sq, D), A_x.dtype),
        scratch_shapes=[
            pltpu.VMEM((1, 1, D), bf16),
            pltpu.VMEM((D,), bf16),
            pltpu.VMEM((R, G, TK, Dh), bf16),
            pltpu.VMEM((D, GD), bf16),
            pltpu.VMEM((H * Dh, D), bf16),
            pltpu.VMEM((F, D), bf16),
            pltpu.VMEM((F, D), bf16),
            pltpu.VMEM((F, D), bf16),
            pltpu.VMEM((1, 1, D), A_x.dtype),
            pltpu.VMEM((NJ, G, TK), f32),
            pltpu.VMEM((G, GD), f32),
            pltpu.VMEM((8, F), f32),
            pltpu.VMEM((8, F), bf16),
            pltpu.VMEM((FV, 128), f32),
            pltpu.VMEM((G, D), f32),
            pltpu.VMEM((8, D), f32),
            pltpu.SemaphoreType.DMA((8,)),
            pltpu.SemaphoreType.DMA((NP * R,)),
            pltpu.SemaphoreType.DMA((NG,)),
        ],
        compiler_params=_compiler_params(),
    )(A_x, A_k_cache, A_v_cache, A_wq, A_wo, B_w_gate.T, B_w_up.T, B_w_down, gate_w)
```
